```python
import os as _os
_os.environ.setdefault("JAX_PLATFORMS", "cpu")
import jax
import jax.numpy as jnp

def _softmax(x, axis=-1):
    return jax.nn.softmax(x, axis=axis)
def _gelu(x):
    return jax.nn.gelu(x, approximate=True)
def _silu(x):
    return jax.nn.silu(x)
def _sigmoid(x):
    return jax.nn.sigmoid(x)
def _layernorm(x, axis=-1, eps=1e-5):
    m = jnp.mean(x, axis=axis, keepdims=True)
    v = jnp.var(x, axis=axis, keepdims=True)
    return (x - m) / jnp.sqrt(v + eps)
def _scatter_add(tgt, idx, src, axis=0):
    return tgt.at[idx].add(src)
def _segment_sum(src, seg, n):
    return jax.ops.segment_sum(src, seg, n)
class _Rng:
    def __init__(self, key):
        self._k = key
    def _next(self):
        self._k, sub = jax.random.split(self._k)
        return sub
    def normal(self, shape):
        return jax.random.normal(self._next(), shape, dtype=jnp.bfloat16)
    def randint(self, lo, hi, shape):
        return jax.random.randint(self._next(), shape, lo, hi, dtype=jnp.int32)
    def uniform(self, shape, lo=0.0, hi=1.0):
        return jax.random.uniform(self._next(), shape, jnp.bfloat16, lo, hi)
    def permutation(self, n):
        return jax.random.permutation(self._next(), n)


kernel_name = 'concat_heads__mha_block_cached__mha_block_cached__near_ridge'

def setup_inputs():
    _rng = _Rng(jax.random.key(int.from_bytes(__import__("os").urandom(4), "little")))
    _w = (lambda a: (lambda t: t.astype(jnp.bfloat16) if jnp.issubdtype(t.dtype, jnp.floating) else t)(jnp.asarray(a)))
    def _A_setup():
        B, Sq, D = 16, 32, 1024
        H, Sk, Dh = 32, 32, 128
        return {
            "x": _w((lambda *s: _rng.normal(s) * 0.8)(B, Sq, D)),
            "k_cache": _w((lambda *s: _rng.normal(s) * 0.8)(B, H, Sk, Dh)),
            "v_cache": _w((lambda *s: _rng.normal(s) * 0.05)(B, H, Sk, Dh)),
            "wq": _w((lambda *s: _rng.normal(s) * 0.8)(D, H * Dh) * (D ** -0.5)),
            "wo": _w((lambda *s: _rng.normal(s) * 0.05)(H * Dh, D) * ((H * Dh) ** -0.5)),
        }
    _A_in = _A_setup()

    def _B_setup():
        B, Sq, D = 16, 32, 1024
        H, Sk, Dh = 32, 32, 128
        return {
            "x": _w((lambda *s: _rng.normal(s) * 0.8)(B, Sq, D)),
            "k_cache": _w((lambda *s: _rng.normal(s) * 0.8)(B, H, Sk, Dh)),
            "v_cache": _w((lambda *s: _rng.normal(s) * 0.05)(B, H, Sk, Dh)),
            "wq": _w((lambda *s: _rng.normal(s) * 0.8)(D, H * Dh) * (D ** -0.5)),
            "wo": _w((lambda *s: _rng.normal(s) * 0.05)(H * Dh, D) * ((H * Dh) ** -0.5)),
        }
    _B_in = _B_setup()

    return {
        "A_x": _A_in["x"],
        "A_k_cache": _A_in["k_cache"],
        "A_v_cache": _A_in["v_cache"],
        "A_wq": _A_in["wq"],
        "A_wo": _A_in["wo"],
        "B_x": _B_in["x"],
        "B_k_cache": _B_in["k_cache"],
        "B_v_cache": _B_in["v_cache"],
        "B_wq": _B_in["wq"],
        "B_wo": _B_in["wo"],
    }

def reference(A_x, A_k_cache, A_v_cache, A_wq, A_wo, B_x, B_k_cache, B_v_cache, B_wq, B_wo):
    def _A_ref(x, k_cache, v_cache, wq, wo):
        B, Sq, D = x.shape
        H, Dh = 32, 128
        q = (lambda x, *d: x.transpose(*d))((x @ wq).reshape(B, Sq, H, Dh), 0, 2, 1, 3)
        scores = jnp.einsum("bhqd,bhkd->bhqk", q, k_cache) * (Dh ** -0.5)
        p = _softmax(scores, axis=-1)
        o = jnp.einsum("bhqk,bhkd->bhqd", p, v_cache)
        return (lambda x, *d: x.transpose(*d))(o, 0, 2, 1, 3).reshape(B, Sq, H * Dh) @ wo

    def _B_ref(x, k_cache, v_cache, wq, wo):
        B, Sq, D = x.shape
        H, Dh = 32, 128
        q = (lambda x, *d: x.transpose(*d))((x @ wq).reshape(B, Sq, H, Dh), 0, 2, 1, 3)
        scores = jnp.einsum("bhqd,bhkd->bhqk", q, k_cache) * (Dh ** -0.5)
        p = _softmax(scores, axis=-1)
        o = jnp.einsum("bhqk,bhkd->bhqd", p, v_cache)
        return (lambda x, *d: x.transpose(*d))(o, 0, 2, 1, 3).reshape(B, Sq, H * Dh) @ wo

    a = _A_ref(A_x, A_k_cache, A_v_cache, A_wq, A_wo)
    b = _B_ref(B_x, B_k_cache, B_v_cache, B_wq, B_wo)
    return jnp.concatenate([a, b], axis=-1)
```

```python
import functools
import jax
import jax.numpy as jnp
from jax import lax
import jax.experimental.pallas as pl
import jax.experimental.pallas.tpu as pltpu

B, SQ, D = 16, 32, 1024
H, SK, DH = 32, 32, 128
M = B * SQ
HG = 4
TN = HG * DH
NG = H // HG
NSTEP = 2 * NG
NC = 4
RB = M // NC
SCALE = DH ** -0.5


def _kernel(ax, ak, av, awq, awo, bx, bk, bv, bwq, bwo, out,
            x_buf, wq_buf, k_buf, v_buf, wo_buf, q_buf, o_buf, acc, stage, sems, xsem, osem):

    A = (ax, ak, av, awq, awo)
    Bs = (bx, bk, bv, bwq, bwo)

    def copies(srcs, g, s):
        _, k, v, wq, wo = srcs
        return (
            pltpu.make_async_copy(wq.at[:, pl.ds(g * TN, TN)], wq_buf.at[s], sems.at[0, s]),
            pltpu.make_async_copy(k.at[:, pl.ds(g * HG, HG)], k_buf.at[s], sems.at[1, s]),
            pltpu.make_async_copy(v.at[:, pl.ds(g * HG, HG)], v_buf.at[s], sems.at[2, s]),
            pltpu.make_async_copy(wo.at[pl.ds(g * TN, TN), :], wo_buf.at[s], sems.at[3, s]),
        )

    xa_copy = pltpu.make_async_copy(ax, x_buf.at[0], xsem.at[0])
    xb_copy = pltpu.make_async_copy(bx, x_buf.at[1], xsem.at[1])
    xa_copy.start()
    for c in copies(A, 0, 0):
        c.start()
    xa_copy.wait()

    lane = lax.broadcasted_iota(jnp.int32, (SK, 128), 1) // 32

    def out_copy(br):
        return pltpu.make_async_copy(stage.at[br], out.at[:, pl.ds(br * D, D)], osem.at[br])

    def step(t, carry):
        br = t // NG
        g = lax.rem(t, NG)
        s = lax.rem(t, 2)

        @pl.when(t == NG)
        def _():
            xb_copy.wait()

        for cp in copies(A, 0, s):
            cp.wait()

        gn = lax.rem(t + 1, NG)

        @pl.when(t + 1 < NG)
        def _():
            for c in copies(A, gn, 1 - s):
                c.start()

        @pl.when(jnp.logical_and(t + 1 >= NG, t + 1 < NSTEP))
        def _():
            for c in copies(Bs, gn, 1 - s):
                c.start()

        @pl.when(t == 2)
        def _():
            xb_copy.start()

        @pl.when(t == NG)
        def _():
            out_copy(0).start()

        def Q(c):
            q = jnp.dot(x_buf[br, pl.ds(c * RB, RB), :], wq_buf[s], preferred_element_type=jnp.float32)
            q_buf[c] = q.astype(jnp.bfloat16)

        def S(c):
            cts = []
            for h in range(HG):
                kst = k_buf[s, pl.ds(c * 4, 4), h].reshape(4 * SK, DH)
                qs = q_buf[c, :, pl.ds(h * DH, DH)]
                st = lax.dot_general(kst, qs, (((1,), (1,)), ((), ())),
                                     preferred_element_type=jnp.float32)
                cc = jnp.where(lane == 0, st[0:32],
                               jnp.where(lane == 1, st[32:64],
                                         jnp.where(lane == 2, st[64:96], st[96:128])))
                mx = jnp.max(cc, axis=0, keepdims=True)
                e = jnp.exp((cc - mx) * SCALE)
                l = jnp.sum(e, axis=0, keepdims=True)
                cts.append(e * (1.0 / l))
            pt = jnp.concatenate(cts, axis=0)
            return pt.T

        def P(c, p):
            for j in range(4):
                pj = p[j * 32:(j + 1) * 32]
                lhs = jnp.concatenate(
                    [jnp.where(lane == h, pj, 0.0) for h in range(HG)], axis=0).astype(jnp.bfloat16)
                vst = v_buf[s, c * 4 + j].reshape(HG * SK, DH)
                o = jnp.dot(lhs, vst, preferred_element_type=jnp.float32)
                for h in range(HG):
                    o_buf[c, pl.ds(j * 32, 32), pl.ds(h * DH, DH)] = (
                        o[h * 32:(h + 1) * 32].astype(jnp.bfloat16))

        def O(c):
            r = jnp.dot(o_buf[c], wo_buf[s], preferred_element_type=jnp.float32)
            rows = pl.ds(c * RB, RB)
            new = jnp.where(g == 0, 0.0, acc[rows, :]) + r
            acc[rows, :] = new
            stage[br, rows, :] = new.astype(jnp.bfloat16)

        Q(0); Q(1)
        p0 = S(0); Q(2); P(0, p0)
        p1 = S(1); Q(3); P(1, p1)
        p2 = S(2); O(0); P(2, p2)
        p3 = S(3); O(1); P(3, p3)
        O(2); O(3)
        return carry

    lax.fori_loop(0, NSTEP, step, 0)
    out_copy(1).start()
    out_copy(0).wait()
    out_copy(1).wait()


@jax.jit
def pallas_concat_heads__mha_block_cached__mha_block_cached__near_ridge_kernel(
    A_x, A_k_cache, A_v_cache, A_wq, A_wo, B_x, B_k_cache, B_v_cache, B_wq, B_wo,
):
    bf = jnp.bfloat16
    any_spec = pl.BlockSpec(memory_space=pl.ANY)
    out = pl.pallas_call(
        _kernel,
        out_shape=jax.ShapeDtypeStruct((M, 2 * D), bf),
        in_specs=[any_spec] * 10,
        out_specs=any_spec,
        scratch_shapes=[
            pltpu.VMEM((2, M, D), bf),
            pltpu.VMEM((2, D, TN), bf),
            pltpu.VMEM((2, B, HG, SK, DH), bf),
            pltpu.VMEM((2, B, HG, SK, DH), bf),
            pltpu.VMEM((2, TN, D), bf),
            pltpu.VMEM((NC, RB, TN), bf),
            pltpu.VMEM((NC, RB, TN), bf),
            pltpu.VMEM((M, D), jnp.float32),
            pltpu.VMEM((2, M, D), bf),
            pltpu.SemaphoreType.DMA((4, 2)),
            pltpu.SemaphoreType.DMA((2,)),
            pltpu.SemaphoreType.DMA((2,)),
        ],
        compiler_params=pltpu.CompilerParams(vmem_limit_bytes=64 * 1024 * 1024),
    )(A_x.reshape(M, D), A_k_cache, A_v_cache, A_wq, A_wo,
      B_x.reshape(M, D), B_k_cache, B_v_cache, B_wq, B_wo)
    return out.reshape(B, SQ, 2 * D)
```

```python
import jax
import jax.numpy as jnp
from jax import lax
import jax.experimental.pallas as pl
import jax.experimental.pallas.tpu as pltpu

B, SQ, D = 16, 32, 1024
H, SK, DH = 32, 32, 128
M = B * SQ
HG = 4
TN = HG * DH
NP = 8
NC = 4
RB = M // NC
NKT = D // DH
OW = D // 4
PAD = 128
SCALE = DH ** -0.5
F32 = jnp.float32
BF16 = jnp.bfloat16
TINY = 0
PLAN = "wide"
TAIL = [256, 128, 64, 64]
QMODE = "cat"
OMODE = "cat"
P0 = 3


def _all(op, g):
    return [(op, g, c) for c in range(4)]


def _ssp(g, a, *fill):
    return [("S", g, a), ("S", g, a + 1), *fill, ("P", g, a), ("P", g, a + 1)]


def _attn(g, f):
    return [f[0]] + _ssp(g, 0, f[1]) + _ssp(g, 2, f[2]) + list(f[3:])


PAIR_OPS = (_all("Q", 0) + _attn(0, _all("Q", 1)) + _attn(1, _all("O", 0)) + _all("O", 1))

_LAST = ([("k", 3, 1), ("v", 3, 1), ("wo", 3, 1), ("k", 4, 2), ("v", 4, 2), ("wo", 4, 2)],
         _ssp(3, 0, ("O", 2, 2)) + _ssp(3, 2, ("O", 2, 3)) + _all("S", 4) + [("O", 3, 0)] + _all("P", 4)
         + _ssp(5, 0, ("O", 3, 1)) + _ssp(5, 2, ("O", 3, 2)) + [("O", 3, 3)] + _all("O", 4) + _all("O", 5))
if PLAN == "wide":
    KPROG = [[1,0,0,0],[1,1,1,0],[2,2,1,1],[3,3,3,3],[5,5,5,5],[8,8,8,8]]
    PHASES = [
        ([("k", 0, 1), ("v", 0, 1), ("wq", 4, 1), ("wo", 0, 1)], _attn(0, _all("Q", 4)) + _all("O", 0)),
        ([("wq", 5, 1), ("k", 1, 1), ("v", 1, 1), ("wo", 1, 1), ("k", 2, 1), ("v", 2, 1), ("wo", 2, 1)],
         _attn(1, _all("Q", 5)) + _attn(2, _all("O", 1)) + _all("O", 2)[:2]),
        _LAST,
    ]
    NQS = 6
else:
    KPROG = [[1, 1], [2, 2], [4, 4], [6, 6], [8, 8]]
    PHASES = [
        ([("wq", 2, 1)], _all("Q", 2)),
        ([("k", 0, 1), ("v", 0, 1), ("wq", 3, 1)], _attn(0, _all("Q", 3))),
        ([("wo", 0, 1), ("k", 1, 1), ("v", 1, 1), ("wo", 1, 1)], _attn(1, _all("O", 0)) + _all("O", 1)),
        ([("k", 2, 1), ("v", 2, 1), ("wo", 2, 1), ("wq", 4, 2)],
         _attn(2, _all("Q", 4)) + _all("Q", 5) + _all("O", 2)[:2]),
        _LAST,
    ]
    NQS = 4
NOS = 3
NKC = len(KPROG)
NG0 = len(KPROG[0])
NPH = len(PHASES)

SEM_CHUNK = 0
SEM_PH = NKC
SEM_PAIR = SEM_PH + NPH
SEM_OUT = SEM_PAIR + (NP - P0)
NSEM = SEM_OUT + 1


def _kernel(ax, ak, av, awq, awo, bx, bk, bv, bwq, bwo, out,
            x_buf, wq_buf, k_buf, v_buf, wo_buf, q_buf, o_buf, qacc, acc, stage, sems):
    srcs = ((ax, ak, av, awq, awo), (bx, bk, bv, bwq, bwo))
    full = pl.ds(0, D)

    def mk(s, d, sem, lvl):
        if TINY and lvl >= TINY:
            return pltpu.make_async_copy(ax.at[pl.ds(0, 16), pl.ds(0, 128)],
                                         wq_buf.at[0, pl.ds(0, 16), pl.ds(D, 128)], sem)
        return pltpu.make_async_copy(s, d, sem)

    def cp(kind, src, lg, n, p, hf, sem, lvl):
        _, k, v, wq, wo = src
        if kind == "wq":
            return mk(wq.at[:, pl.ds(lg * TN, n * TN)], wq_buf.at[p, :, pl.ds(hf * TN, n * TN)], sem, lvl)
        if kind == "k":
            return mk(k.at[:, pl.ds(lg * HG, n * HG)], k_buf.at[p, :, pl.ds(hf * HG, n * HG)], sem, lvl)
        if kind == "v":
            return mk(v.at[:, pl.ds(lg * HG, n * HG)], v_buf.at[p, :, pl.ds(hf * HG, n * HG)], sem, lvl)
        return mk(wo.at[pl.ds(lg * TN, n * TN), :], wo_buf.at[p, pl.ds(hf * TN, n * TN), full], sem, lvl)

    def cp_x(br, kt, sem, lvl):
        return mk(srcs[br][0].at[:, pl.ds(kt * DH, DH)], x_buf.at[br, kt], sem, lvl)

    def kranges(i):
        prev = KPROG[i - 1] if i else [0] * NG0
        return list(zip(prev, KPROG[i]))

    def cp_chunk(i):
        sem = sems.at[SEM_CHUNK + i]
        kr = kranges(i)
        cps = [cp_x(0, kt, sem, 1) for kt in range(max(a for a, _ in kr), max(b for _, b in kr))]
        g = 0
        while g < NG0:
            n = 2 if (g % 2 == 0 and kr[g] == kr[g + 1]) else 1
            a, b = kr[g]
            if b > a:
                ks = pl.ds(a * DH, (b - a) * DH)
                cps.append(mk(awq.at[ks, pl.ds(g * TN, n * TN)],
                              wq_buf.at[g // 2, ks, pl.ds((g % 2) * TN, n * TN)], sem, 1))
            g += n
        return cps

    def cp_pair(src, lp, p, sem):
        return [cp(kind, src, 2 * lp, 2, p, 0, sem, 3) for kind in ("wq", "k", "v", "wo")]

    def cp_xb():
        return [cp_x(1, kt, sems.at[SEM_PAIR + (NP // 2 - P0)], 3) for kt in range(NKT)]

    def out_pieces(n):
        sizes = TAIL if n == 3 else [M]
        return [(sum(sizes[:i]), sizes[i]) for i in range(len(sizes))]

    def cp_out(br, n, r0, nr):
        rows = pl.ds(r0, nr)
        return pltpu.make_async_copy(stage.at[br, rows, pl.ds(n * OW, OW)],
                                     out.at[rows, pl.ds(br * D + n * OW, OW)], sems.at[SEM_OUT])

    chunks = [cp_chunk(i) for i in range(NKC)]
    phase_cps = [[cp(kind, srcs[0], g, n, g // 2, g % 2, sems.at[SEM_PH + i], 2) for kind, g, n in data]
                 for i, (data, _) in enumerate(PHASES)]
    ndma = 0
    for cps in chunks + phase_cps:
        for c in cps:
            c.start(); ndma += 1
    for p in range(P0, NP):
        cps = cp_pair(srcs[p // (NP // 2)], p % (NP // 2), p, sems.at[SEM_PAIR + p - P0])
        if p == NP // 2:
            cps = cp_xb() + cps
        for c in cps:
            c.start(); ndma += 1

    lane = lax.broadcasted_iota(jnp.int32, (SK, 128), 1) // 32

    def x_tiles(br, a, b):
        return jnp.concatenate([x_buf[br, kt] for kt in range(a, b)], axis=1)

    def Q(br, p, hf, qs, h):
        if QMODE == "sum":
            q = None
            for kt in range(NKT):
                r = jnp.dot(x_buf[br, kt], wq_buf[p, pl.ds(kt * DH, DH), pl.ds(hf * TN + h * DH, DH)],
                            preferred_element_type=F32)
                q = r if q is None else q + r
        else:
            q = jnp.dot(x_tiles(br, 0, NKT), wq_buf[p, :, pl.ds(hf * TN + h * DH, DH)], preferred_element_type=F32)
        q_buf[qs, h] = q.astype(BF16)

    def S(p, hf, qs, c):
        cts = []
        for h in range(HG):
            kst = k_buf[p, pl.ds(c * 4, 4), hf * HG + h].reshape(4 * SK, DH)
            qh = q_buf[qs, h, pl.ds(c * RB, RB), :]
            st = lax.dot_general(kst, qh, (((1,), (1,)), ((), ())),
                                 preferred_element_type=F32)
            cc = jnp.where(lane == 0, st[0:32],
                           jnp.where(lane == 1, st[32:64],
                                     jnp.where(lane == 2, st[64:96], st[96:128])))
            mx = jnp.max(cc, axis=0, keepdims=True)
            e = jnp.exp((cc - mx) * SCALE)
            l = jnp.sum(e, axis=0, keepdims=True)
            cts.append(e * (1.0 / l))
        pt = jnp.concatenate(cts, axis=0)
        return pt.T

    def P(p, hf, os_, c, pr):
        for j in range(4):
            pj = pr[j * 32:(j + 1) * 32]
            lhs = jnp.concatenate(
                [jnp.where(lane == h, pj, 0.0) for h in range(HG)], axis=0).astype(BF16)
            vst = v_buf[p, c * 4 + j, pl.ds(hf * HG, HG)].reshape(HG * SK, DH)
            o = jnp.dot(lhs, vst, preferred_element_type=F32)
            for h in range(HG):
                o_buf[os_, h, pl.ds(c * RB + j * 32, 32), :] = o[h * 32:(h + 1) * 32].astype(BF16)

    def O(p, hf, os_, n, first, last_fn=None):
        cols = pl.ds(n * OW, OW)
        if OMODE == "sum":
            rs = []
            for t in range(OW // DH):
                r = None
                for h in range(HG):
                    rr = jnp.dot(o_buf[os_, h], wo_buf[p, pl.ds(hf * TN + h * DH, DH), pl.ds(n * OW + t * DH, DH)],
                                 preferred_element_type=F32)
                    r = rr if r is None else r + rr
                rs.append(r)
            r = jnp.concatenate(rs, axis=1)
        else:
            o = jnp.concatenate([o_buf[os_, h] for h in range(HG)], axis=1)
            r = jnp.dot(o, wo_buf[p, pl.ds(hf * TN, TN), cols], preferred_element_type=F32)
        if first is True:
            new = r
        elif first is False:
            new = acc[:, cols] + r
        else:
            new = jnp.where(first, 0.0, acc[:, cols]) + r
        acc[:, cols] = new
        if last_fn is not None:
            last_fn(n, new)

    def run(ops, br, pair_of, first_of, last_of):
        probs = {}
        for op, g, c in ops:
            p, hf = pair_of(g), g % 2
            if op == "Q":
                Q(br, p, hf, g % NQS, c)
            elif op == "S":
                probs[g, c] = S(p, hf, g % NQS, c)
            elif op == "P":
                P(p, hf, g % NOS, c, probs.pop((g, c)))
            else:
                O(p, hf, g % NOS, c, first_of(g), last_of(g))
        assert not probs

    def wait_all(cps):
        for c in cps:
            c.wait()

    for i in range(NKC):
        wait_all(chunks[i])
        for g, (a, b) in enumerate(kranges(i)):
            if b == a:
                continue
            r = jnp.dot(x_tiles(0, a, b), wq_buf[g // 2, pl.ds(a * DH, (b - a) * DH), pl.ds((g % 2) * TN, TN)],
                        preferred_element_type=F32)
            if a > 0:
                r = r + qacc[g]
            if b < NKT:
                qacc[g] = r
            else:
                rb = r.astype(BF16)
                for h in range(HG):
                    q_buf[g, h] = rb[:, h * DH:(h + 1) * DH]
    for i, (_, ops) in enumerate(PHASES):
        wait_all(phase_cps[i])
        run(ops, 0, lambda g: g // 2, lambda g: g == 0, lambda g: None)

    def pair_step(p, carry):
        @pl.when(p == NP // 2)
        def _():
            wait_all(cp_xb())

        wait_all(cp_pair(srcs[0], 0, p, sems.at[SEM_PAIR + p - P0]))
        br = lax.shift_right_logical(p, 2)

        def last_fn(n, new):
            nb = new.astype(BF16)
            for r0, nr in out_pieces(n):
                stage[br, pl.ds(r0, nr), pl.ds(n * OW, OW)] = nb[r0:r0 + nr]
                for b in range(2):
                    @pl.when(p == (b + 1) * (NP // 2) - 1)
                    def _():
                        cp_out(b, n, r0, nr).start()

        run(PAIR_OPS, br, lambda g: p, lambda g: (p == NP // 2) if g == 0 else False,
            lambda g: last_fn if g == 1 else None)
        return carry

    lax.fori_loop(P0, NP, pair_step, 0)
    for br in range(2):
        for n in range(4):
            for r0, nr in out_pieces(n):
                cp_out(br, n, r0, nr).wait()


@jax.jit
def pallas_concat_heads__mha_block_cached__mha_block_cached__near_ridge_kernel(
    A_x, A_k_cache, A_v_cache, A_wq, A_wo, B_x, B_k_cache, B_v_cache, B_wq, B_wo,
):
    any_spec = pl.BlockSpec(memory_space=pl.ANY)
    out = pl.pallas_call(
        _kernel,
        out_shape=jax.ShapeDtypeStruct((M, 2 * D), BF16),
        in_specs=[any_spec] * 10,
        out_specs=any_spec,
        scratch_shapes=[
            pltpu.VMEM((2, NKT, M, DH), BF16),
            pltpu.VMEM((NP, D, 2 * TN + PAD), BF16),
            pltpu.VMEM((NP, B, 2 * HG, SK, DH), BF16),
            pltpu.VMEM((NP, B, 2 * HG, SK, DH), BF16),
            pltpu.VMEM((NP, 2 * TN, D + PAD), BF16),
            pltpu.VMEM((NQS, HG, M, DH), BF16),
            pltpu.VMEM((NOS, HG, M, DH), BF16),
            pltpu.VMEM((NG0, M, TN), F32),
            pltpu.VMEM((M, D), F32),
            pltpu.VMEM((2, M, D), BF16),
            pltpu.SemaphoreType.DMA((NSEM,)),
        ],
        compiler_params=pltpu.CompilerParams(vmem_limit_bytes=100 * 1024 * 1024,
                                             disable_semaphore_checks=True),
    )(A_x.reshape(M, D), A_k_cache, A_v_cache, A_wq, A_wo,
      B_x.reshape(M, D), B_k_cache, B_v_cache, B_wq, B_wo)
    return out.reshape(B, SQ, 2 * D)
```

```python
import jax
import jax.numpy as jnp
from jax import lax
import jax.experimental.pallas as pl
import jax.experimental.pallas.tpu as pltpu

B, SQ, D = 16, 32, 1024
H, SK, DH = 32, 32, 128
M = B * SQ
HG = 4
TN = HG * DH
NP = 8
NPB = NP // 2
RB = 4 * SQ
NKT = D // DH
OW = D // 4
PAD = 128
SCALE = DH ** -0.5
F32 = jnp.float32
BF16 = jnp.bfloat16
NQS, NOS = 6, 3
P0 = 3


def _all(op, g):
    return [(op, g, c) for c in range(4)]


def _ssp(g, a, fill):
    return [("S", g, a), ("S", g, a + 1), fill, ("P", g, a), ("P", g, a + 1)]


def _attn(g, f):
    return [f[0]] + _ssp(g, 0, f[1]) + _ssp(g, 2, f[2]) + [f[3]]


PAIR_OPS = _all("Q", 0) + _attn(0, _all("Q", 1)) + _attn(1, _all("O", 0)) + _all("O", 1)

KPROG = ((1, 0, 0, 0), (1, 1, 1, 0), (2, 2, 1, 1), (3, 3, 3, 3), (5, 5, 5, 5), (8, 8, 8, 8))
NG0 = len(KPROG[0])
PHASES = (
    ((("k", 0, 1), ("v", 0, 1), ("wq", 4, 1), ("wo", 0, 1)),
     _attn(0, _all("Q", 4)) + _all("O", 0)),
    ((("wq", 5, 1), ("k", 1, 1), ("v", 1, 1), ("wo", 1, 1), ("k", 2, 1), ("v", 2, 1), ("wo", 2, 1)),
     _attn(1, _all("Q", 5)) + _attn(2, _all("O", 1)) + _all("O", 2)[:2]),
    ((("k", 3, 1), ("v", 3, 1), ("wo", 3, 1), ("k", 4, 2), ("v", 4, 2), ("wo", 4, 2)),
     _ssp(3, 0, ("O", 2, 2)) + _ssp(3, 2, ("O", 2, 3)) + _all("S", 4) + [("O", 3, 0)] + _all("P", 4)
     + _ssp(5, 0, ("O", 3, 1)) + _ssp(5, 2, ("O", 3, 2)) + [("O", 3, 3)] + _all("O", 4) + _all("O", 5)),
)
TAIL = (128, 128, 128, 64, 32, 32)

SEM_CHUNK = 0
SEM_PH = SEM_CHUNK + len(KPROG)
SEM_PAIR = SEM_PH + len(PHASES)
SEM_OUT = SEM_PAIR + (NP - P0)
NSEM = SEM_OUT + 1


def _out_pieces(n):
    if n < 3:
        return [(0, M, n * OW, OW)]
    return [(0, M, n * OW, DH)] + [(sum(TAIL[:i]), TAIL[i], n * OW + DH, DH) for i in range(len(TAIL))]


def _kernel(ax, ak, av, awq, awo, bx, bk, bv, bwq, bwo, out,
            x_buf, wq_buf, k_buf, v_buf, wo_buf, q_buf, o_buf, qacc, acc, stage, sems):
    srcs = ((ax, ak, av, awq, awo), (bx, bk, bv, bwq, bwo))
    copy = pltpu.make_async_copy

    def cp(kind, src, lg, n, p, hf, sem):
        _, k, v, wq, wo = src
        if kind == "wq":
            return copy(wq.at[:, pl.ds(lg * TN, n * TN)], wq_buf.at[p, :, pl.ds(hf * TN, n * TN)], sem)
        if kind == "k":
            return copy(k.at[:, pl.ds(lg * HG, n * HG)], k_buf.at[p, :, pl.ds(hf * HG, n * HG)], sem)
        if kind == "v":
            return copy(v.at[:, pl.ds(lg * HG, n * HG)], v_buf.at[p, :, pl.ds(hf * HG, n * HG)], sem)
        return copy(wo.at[pl.ds(lg * TN, n * TN), :], wo_buf.at[p, pl.ds(hf * TN, n * TN), pl.ds(0, D)], sem)

    def cp_x(br, kt, sem):
        return copy(srcs[br][0].at[:, pl.ds(kt * DH, DH)], x_buf.at[br, kt], sem)

    def kranges(i):
        return list(zip(KPROG[i - 1] if i else (0,) * NG0, KPROG[i]))

    def cp_chunk(i):
        sem = sems.at[SEM_CHUNK + i]
        kr = kranges(i)
        cps = [cp_x(0, kt, sem) for kt in range(max(a for a, _ in kr), max(b for _, b in kr))]
        g = 0
        while g < NG0:
            n = 2 if (g % 2 == 0 and kr[g] == kr[g + 1]) else 1
            a, b = kr[g]
            if b > a:
                ks = pl.ds(a * DH, (b - a) * DH)
                cps.append(copy(awq.at[ks, pl.ds(g * TN, n * TN)],
                                wq_buf.at[g // 2, ks, pl.ds((g % 2) * TN, n * TN)], sem))
            g += n
        return cps

    def cp_pair(br, lp, p):
        sem = sems.at[SEM_PAIR + p - P0]
        return [cp(kind, srcs[br], 2 * lp, 2, p, 0, sem) for kind in ("wq", "k", "v", "wo")]

    def cp_xb():
        return [cp_x(1, kt, sems.at[SEM_PAIR + NPB - P0]) for kt in range(NKT)]

    def cp_out(br, r0, nr, c0, nc):
        rows = pl.ds(r0, nr)
        return copy(stage.at[br, rows, pl.ds(c0, nc)], out.at[rows, pl.ds(br * D + c0, nc)], sems.at[SEM_OUT])

    def wait_all(cps):
        for c in cps:
            c.wait()

    chunk_cps = [cp_chunk(i) for i in range(len(KPROG))]
    phase_cps = [[cp(kind, srcs[0], g, n, g // 2, g % 2, sems.at[SEM_PH + i]) for kind, g, n in data]
                 for i, (data, _) in enumerate(PHASES)]
    pair_cps = [(cp_xb() if p == NPB else []) + cp_pair(p // NPB, p % NPB, p) for p in range(P0, NP)]
    for cps in chunk_cps + phase_cps + pair_cps:
        for c in cps:
            c.start()

    lane = lax.broadcasted_iota(jnp.int32, (SK, 128), 1) // SK

    def x_tiles(br, a, b):
        return jnp.concatenate([x_buf[br, kt] for kt in range(a, b)], axis=1)

    def q_proj(br, p, hf, qs, h):
        q = jnp.dot(x_tiles(br, 0, NKT), wq_buf[p, :, pl.ds(hf * TN + h * DH, DH)], preferred_element_type=F32)
        q_buf[qs, h] = q.astype(BF16)

    def scores(p, hf, qs, c):
        pts = []
        for h in range(HG):
            kst = k_buf[p, pl.ds(c * 4, 4), hf * HG + h].reshape(4 * SK, DH)
            qh = q_buf[qs, h, pl.ds(c * RB, RB), :]
            st = lax.dot_general(kst, qh, (((1,), (1,)), ((), ())),
                                 preferred_element_type=F32)
            s = jnp.where(lane == 0, st[0:32],
                          jnp.where(lane == 1, st[32:64],
                                    jnp.where(lane == 2, st[64:96], st[96:128])))
            mx = jnp.max(s, axis=0, keepdims=True)
            e = jnp.exp((s - mx) * SCALE)
            l = jnp.sum(e, axis=0, keepdims=True)
            pts.append(e * (1.0 / l))
        return jnp.concatenate(pts, axis=0).T

    def values(p, hf, os_, c, pr):
        for j in range(4):
            pj = pr[j * SQ:(j + 1) * SQ]
            lhs = jnp.concatenate(
                [jnp.where(lane == h, pj, 0.0) for h in range(HG)], axis=0).astype(BF16)
            vst = v_buf[p, c * 4 + j, pl.ds(hf * HG, HG)].reshape(HG * SK, DH)
            o = jnp.dot(lhs, vst, preferred_element_type=F32)
            for h in range(HG):
                o_buf[os_, h, pl.ds(c * RB + j * SQ, SQ), :] = o[h * SQ:(h + 1) * SQ].astype(BF16)

    def o_proj(p, hf, os_, n, first, emit):
        cols = pl.ds(n * OW, OW)
        o = jnp.concatenate([o_buf[os_, h] for h in range(HG)], axis=1)
        r = jnp.dot(o, wo_buf[p, pl.ds(hf * TN, TN), cols], preferred_element_type=F32)
        if first is False:
            r = acc[:, cols] + r
        elif first is not True:
            r = jnp.where(first, 0.0, acc[:, cols]) + r
        acc[:, cols] = r
        if emit is not None:
            emit(n, r)

    def run(ops, br, pair_of, first_of, emit_of):
        probs = {}
        for op, g, c in ops:
            p, hf = pair_of(g), g % 2
            if op == "Q":
                q_proj(br, p, hf, g % NQS, c)
            elif op == "S":
                probs[g, c] = scores(p, hf, g % NQS, c)
            elif op == "P":
                values(p, hf, g % NOS, c, probs.pop((g, c)))
            else:
                o_proj(p, hf, g % NOS, c, first_of(g), emit_of(g))

    for i in range(len(KPROG)):
        wait_all(chunk_cps[i])
        for g, (a, b) in enumerate(kranges(i)):
            if b == a:
                continue
            r = jnp.dot(x_tiles(0, a, b), wq_buf[g // 2, pl.ds(a * DH, (b - a) * DH), pl.ds((g % 2) * TN, TN)],
                        preferred_element_type=F32)
            if a > 0:
                r = r + qacc[g]
            if b < NKT:
                qacc[g] = r
            else:
                rb = r.astype(BF16)
                for h in range(HG):
                    q_buf[g, h] = rb[:, h * DH:(h + 1) * DH]
    for i, (_, ops) in enumerate(PHASES):
        wait_all(phase_cps[i])
        run(ops, 0, lambda g: g // 2, lambda g: g == 0, lambda g: None)

    def pair_step(p, carry):
        @pl.when(p == NPB)
        def _():
            wait_all(cp_xb())

        wait_all(cp_pair(0, 0, p))

        @pl.when(p == NPB)
        def _():
            cp_out(0, 0, M, 0, D).start()

        br = lax.shift_right_logical(p, 2)

        def emit(n, r):
            for r0, nr, c0, nc in _out_pieces(n):
                lo = c0 - n * OW
                stage[br, pl.ds(r0, nr), pl.ds(c0, nc)] = r[r0:r0 + nr, lo:lo + nc].astype(BF16)

                @pl.when(p == NP - 1)
                def _():
                    cp_out(1, r0, nr, c0, nc).start()

        run(PAIR_OPS, br, lambda g: p, lambda g: (p == NPB) if g == 0 else False,
            lambda g: emit if g == 1 else None)
        return carry

    lax.fori_loop(P0, NP, pair_step, 0)
    cp_out(0, 0, M, 0, D).wait()
    for n in range(4):
        for piece in _out_pieces(n):
            cp_out(1, *piece).wait()


@jax.jit
def pallas_concat_heads__mha_block_cached__mha_block_cached__near_ridge_kernel(
    A_x: jax.Array,
    A_k_cache: jax.Array,
    A_v_cache: jax.Array,
    A_wq: jax.Array,
    A_wo: jax.Array,
    B_x: jax.Array,
    B_k_cache: jax.Array,
    B_v_cache: jax.Array,
    B_wq: jax.Array,
    B_wo: jax.Array,
):
    any_spec = pl.BlockSpec(memory_space=pl.ANY)
    out = pl.pallas_call(
        _kernel,
        out_shape=jax.ShapeDtypeStruct((M, 2 * D), BF16),
        in_specs=[any_spec] * 10,
        out_specs=any_spec,
        scratch_shapes=[
            pltpu.VMEM((2, NKT, M, DH), BF16),
            pltpu.VMEM((NP, D, 2 * TN + PAD), BF16),
            pltpu.VMEM((NP, B, 2 * HG, SK, DH), BF16),
            pltpu.VMEM((NP, B, 2 * HG, SK, DH), BF16),
            pltpu.VMEM((NP, 2 * TN, D + PAD), BF16),
            pltpu.VMEM((NQS, HG, M, DH), BF16),
            pltpu.VMEM((NOS, HG, M, DH), BF16),
            pltpu.VMEM((NG0, M, TN), F32),
            pltpu.VMEM((M, D), F32),
            pltpu.VMEM((2, M, D), BF16),
            pltpu.SemaphoreType.DMA((NSEM,)),
        ],
        compiler_params=pltpu.CompilerParams(vmem_limit_bytes=100 * 1024 * 1024,
                                             disable_semaphore_checks=True),
    )(A_x.reshape(M, D), A_k_cache, A_v_cache, A_wq, A_wo,
      B_x.reshape(M, D), B_k_cache, B_v_cache, B_wq, B_wo)
    return out.reshape(B, SQ, 2 * D)
```

```python
import jax
import jax.numpy as jnp
from jax import lax
import jax.experimental.pallas as pl
import jax.experimental.pallas.tpu as pltpu

B, SQ, D = 16, 32, 1024
H, SK, DH = 32, 32, 128
M = B * SQ
HG = 4
TN = HG * DH
NP = 8
NPB = NP // 2
RB = 4 * SQ
NKT = D // DH
PAD = 128
SCALE = DH ** -0.5
F32 = jnp.float32
BF16 = jnp.bfloat16
U32 = jnp.uint32
NQS, NOS = 6, 2
P0 = 3
OMIX = 0

OQ_M = ((0, 256, 0, 512), (0, 256, 512, 512), (256, 256, 0, 512), (256, 256, 512, 512))
OQ_X = ((0, 256, 0, 512), (256, 256, 0, 512), (0, 512, 512, 256), (0, 512, 768, 256))


def _chain(blocks, fills, prev=None):
    ops = []
    for b, f in zip(blocks, fills):
        ops += [("S", b, None) if prev is None else ("C", b, prev), f]
        prev = b
    return ops


def _blocks(*gs):
    return [(g, c) for g in gs for c in range(4)]


def _q(g):
    return [("Q", g, h) for h in range(4)]


def _o(g, oq=OQ_M):
    return [("O", g, q) for q in oq]


PAIR_OPS = (_q(0) + _q(1)[:1] + _chain(_blocks(0, 1), _q(1)[1:] + _o(0) + _o(1)[:1])
            + [("P", None, (1, 3))] + _o(1)[1:])

KPROG = ((1,0,0,0,0),(1,1,1,0,0),(2,1,1,1,1),(3,3,2,2,2),(5,5,4,4,4),(8,8,8,8,7),(8,8,8,8,8))
NG0 = len(KPROG[0])
_OS = OQ_X if OMIX else OQ_M
PHASES = (
    ((("k", 0, 1), ("wq", 5, 1), ("v", 0, 1), ("k", 1, 1), ("wo", 0, 1), ("v", 1, 1)),
     _chain(_blocks(0, 1), _q(5) + _o(0, _OS))),
    ((("k", 2, 2), ("v", 2, 2), ("wo", 1, 1), ("wo", 2, 1)),
     _chain(_blocks(2, 3), _o(1, _OS) + _o(2, _OS), (1, 3))),
    ((("k", 4, 2), ("v", 4, 2), ("wo", 3, 1), ("wo", 4, 2)),
     _chain(_blocks(4, 5), _o(3, _OS) + _o(4, _OS), (3, 3)) + [("P", None, (5, 3))] + _o(5, _OS)),
)
NCH = len(KPROG)
NPHASE = NCH - 1 + len(PHASES)
TAIL = (128, 64, 32, 32)

SEM_PAIR = NPHASE
SEM_OUT = SEM_PAIR + (NP - P0)
NSEM = SEM_OUT + 1


def _out_pieces(q):
    r0, nr, c0, nc = q
    if q != OQ_M[-1]:
        return [q]
    last = c0 + nc - DH
    return ([(r0, nr, c, DH) for c in range(c0, last, DH)]
            + [(r0 + sum(TAIL[:i]), TAIL[i], last, DH) for i in range(len(TAIL))])


def _kernel(ax, ak, av, awq, awo, bx, bk, bv, bwq, bwo, out,
            x_buf, wq_buf, k_buf, v_buf, wo_buf, qt_buf, o_buf, qacc, acc, stage, sems):
    srcs = ((ax, ak, av, awq, awo), (bx, bk, bv, bwq, bwo))

    copy = pltpu.make_async_copy

    def cp(kind, src, lg, n, p, hf, sem):
        _, k, v, wq, wo = src
        if kind == "wq":
            return copy(wq.at[:, pl.ds(lg * TN, n * TN)], wq_buf.at[p, :, pl.ds(hf * TN, n * TN)], sem)
        if kind == "k":
            return copy(k.at[:, pl.ds(lg * HG, n * HG)], k_buf.at[p, :, pl.ds(hf * HG, n * HG)], sem)
        if kind == "v":
            return copy(v.at[:, pl.ds(lg * HG, n * HG)], v_buf.at[p, :, pl.ds(hf * HG, n * HG)], sem)
        return copy(wo.at[pl.ds(lg * TN, n * TN), :], wo_buf.at[p, pl.ds(hf * TN, n * TN), pl.ds(0, D)], sem)

    def cp_x(br, kt, sem):
        return copy(srcs[br][0].at[:, pl.ds(kt * DH, DH)], x_buf.at[br, kt], sem)

    def kranges(i):
        return list(zip(KPROG[i - 1] if i else (0,) * NG0, KPROG[i]))

    def cp_chunk(i):
        sem = sems.at[i]
        kr = kranges(i)
        cps = [cp_x(0, kt, sem) for kt in range(max(a for a, _ in kr), max(b for _, b in kr))]
        g = 0
        while g < NG0:
            n = 2 if (g % 2 == 0 and g + 1 < NG0 and kr[g] == kr[g + 1]) else 1
            a, b = kr[g]
            if b > a:
                ks = pl.ds(a * DH, (b - a) * DH)
                cps.append(copy(awq.at[ks, pl.ds(g * TN, n * TN)],
                                wq_buf.at[g // 2, ks, pl.ds((g % 2) * TN, n * TN)], sem))
            g += n
        return cps

    def cp_pair(br, lp, p):
        sem = sems.at[SEM_PAIR + p - P0]
        return [cp(kind, srcs[br], 2 * lp, 2, p, 0, sem) for kind in ("wq", "k", "v", "wo")]

    def cp_xb():
        return [cp_x(1, kt, sems.at[SEM_PAIR + NPB - P0]) for kt in range(NKT)]

    def cp_out(br, r0, nr, c0, nc):
        rows = pl.ds(r0, nr)
        return pltpu.make_async_copy(stage.at[br, rows, pl.ds(c0, nc)], out.at[rows, pl.ds(br * D + c0, nc)],
                                     sems.at[SEM_OUT])

    def wait_all(cps):
        for c in cps:
            c.wait()

    phase_cps = [cp_chunk(i) if i < NCH else [] for i in range(NPHASE)]
    for i, (data, _) in enumerate(PHASES):
        ph = NCH - 1 + i
        phase_cps[ph] += [cp(kind, srcs[0], g, n, g // 2, g % 2, sems.at[ph]) for kind, g, n in data]
    pair_cps = [(cp_xb() if p == NPB else []) + cp_pair(p // NPB, p % NPB, p) for p in range(P0, NP)]
    for cps in phase_cps + pair_cps:
        for c in cps:
            c.start()

    lane = lax.broadcasted_iota(jnp.int32, (SK, 128), 1) // SK
    lane2 = lax.broadcasted_iota(jnp.int32, (SK // 2, 128), 1) // SK
    zero2 = jnp.zeros((SK // 2, 128), U32)
    packed = lambda a: pltpu.bitcast(a, U32)
    unpacked = lambda a: pltpu.bitcast(a, BF16)
    keep = lambda j, a: jnp.where(lane2 != j, zero2, a)
    drop = lambda j, a: jnp.where(lane2 == j, zero2, a)
    sel = lambda j, a, b: jnp.where(lane2 == j, a, b)

    def x_tiles(br, a, b):
        return jnp.concatenate([x_buf[br, kt] for kt in range(a, b)], axis=1)

    def store_q(slot, h, q):
        for c in range(4):
            qt_buf[slot, h, c] = packed(q[c * RB:(c + 1) * RB].T.astype(BF16))

    def softmax_t(ss):
        pts = []
        for s in ss:
            mx = jnp.max(s, axis=0, keepdims=True)
            e = jnp.exp((s - mx) * SCALE)
            l = jnp.sum(e, axis=0, keepdims=True)
            pts.append(e * (1.0 / l))
        return packed(jnp.concatenate(pts, axis=0).T.astype(BF16))

    def dot(a, rows):
        return jnp.dot(unpacked(a), unpacked(jnp.concatenate(rows, axis=0)), preferred_element_type=F32)

    def run(ops, br, pair_of, first_of, emit_of, probs):
        for op, a, b in ops:
            if op == "Q":
                g, h = a, b
                q = jnp.dot(x_tiles(br, 0, NKT), wq_buf[pair_of(g), :, pl.ds((g % 2) * TN + h * DH, DH)],
                            preferred_element_type=F32)
                store_q(g % NQS, h, q)
                continue
            if op == "O":
                g, (r0, nr, c0, nc) = a, b
                rows, cols = pl.ds(r0, nr), pl.ds(c0, nc)
                o = jnp.concatenate([o_buf[g % NOS, h, rows, :] for h in range(HG)], axis=1)
                r = jnp.dot(o, wo_buf[pair_of(g), pl.ds((g % 2) * TN, TN), cols], preferred_element_type=F32)
                first = first_of(g)
                if first is False:
                    r = acc[rows, cols] + r
                elif first is not True:
                    r = jnp.where(first, 0.0, acc[rows, cols]) + r
                acc[rows, cols] = r
                if emit_of(g) is not None:
                    emit_of(g)(b, r)
                continue
            if a is not None:
                gs, cs = a
                kk = lambda i, j: packed(k_buf[pair_of(gs), cs * 4 + j, (gs % 2) * HG + i])
                qt = lambda i, r: qt_buf[gs % NQS, i, cs, pl.ds(r * (SK // 2), SK // 2), :]
            if b is not None:
                gp, cp_ = b
                vv = lambda i, r: packed(v_buf[pair_of(gp), cp_ * 4 + i, (gp % 2) * HG + r])
                pr = probs.pop(b)
                pc = [pr[i * (SQ // 2):(i + 1) * (SQ // 2)] for i in range(4)]

                def put_o(i, j, o):
                    o_buf[gp % NOS, j, pl.ds(cp_ * RB + i * SQ, SQ), :] = o.astype(BF16)
            if op == "S":
                ss = []
                for i in range(4):
                    st = dot(jnp.concatenate([kk(i, j) for j in range(4)], axis=0), [qt(i, r) for r in range(4)])
                    ss.append(jnp.where(lane == 0, st[0:32], jnp.where(
                        lane == 1, st[32:64], jnp.where(lane == 2, st[64:96], st[96:128]))))
                probs[a] = softmax_t(ss)
            elif op == "P":
                for i in range(4):
                    o = dot(jnp.concatenate([keep(j, pc[i]) for j in range(4)], axis=0), [vv(i, r) for r in range(4)])
                    for j in range(4):
                        put_o(i, j, o[j * SQ:(j + 1) * SQ])
            else:
                ss = [dot(sel(0, kk(i, 0), sel(1, kk(i, 1), sel(2, kk(i, 2), kk(i, 3)))),
                          [keep(r, qt(i, r)) for r in range(4)]) for i in range(4)]
                od = [dot(pc[i], [keep(r, vv(i, r)) for r in range(4)]) for i in range(4)]
                for j in range(4):
                    for i in range(4):
                        t = dot(sel(j, pc[i], kk(i, j)),
                                [drop(j, vv(i, r)) if r == j else keep(j, qt(i, r)) for r in range(4)])
                        put_o(i, j, jnp.where(lane == j, od[i], t))
                        ss[i] = jnp.where(lane == j, ss[i] + t, ss[i])
                probs[a] = softmax_t(ss)

    probs0 = {}
    for ph in range(NPHASE):
        wait_all(phase_cps[ph])
        if ph < NCH:
            for g, (a, b) in enumerate(kranges(ph)):
                if b == a:
                    continue
                r = jnp.dot(x_tiles(0, a, b), wq_buf[g // 2, pl.ds(a * DH, (b - a) * DH), pl.ds((g % 2) * TN, TN)],
                            preferred_element_type=F32)
                if a > 0:
                    r = r + qacc[g]
                if b < NKT:
                    qacc[g] = r
                else:
                    for h in range(HG):
                        store_q(g, h, r[:, h * DH:(h + 1) * DH])
        if ph >= NCH - 1:
            run(PHASES[ph - (NCH - 1)][1], 0, lambda g: g // 2, lambda g: g == 0, lambda g: None, probs0)

    def pair_step(p, carry):
        @pl.when(p == NPB)
        def _():
            wait_all(cp_xb())

        wait_all(cp_pair(0, 0, p))

        @pl.when(p == NPB)
        def _():
            cp_out(0, 0, M, 0, D).start()

        br = lax.shift_right_logical(p, 2)

        def emit(q, r):
            for r0, nr, c0, nc in _out_pieces(q):
                stage[br, pl.ds(r0, nr), pl.ds(c0, nc)] = (
                    r[r0 - q[0]:r0 - q[0] + nr, c0 - q[2]:c0 - q[2] + nc].astype(BF16))

                @pl.when(p == NP - 1)
                def _():
                    cp_out(1, r0, nr, c0, nc).start()

        run(PAIR_OPS, br, lambda g: p, lambda g: (p == NPB) if g == 0 else False,
            lambda g: emit if g == 1 else None, {})
        return carry

    lax.fori_loop(P0, NP, pair_step, 0)
    cp_out(0, 0, M, 0, D).wait()
    for q in OQ_M:
        for piece in _out_pieces(q):
            cp_out(1, *piece).wait()


@jax.jit
def pallas_concat_heads__mha_block_cached__mha_block_cached__near_ridge_kernel(
    A_x, A_k_cache, A_v_cache, A_wq, A_wo, B_x, B_k_cache, B_v_cache, B_wq, B_wo,
):
    any_spec = pl.BlockSpec(memory_space=pl.ANY)
    out = pl.pallas_call(
        _kernel,
        out_shape=jax.ShapeDtypeStruct((M, 2 * D), BF16),
        in_specs=[any_spec] * 10,
        out_specs=any_spec,
        scratch_shapes=[
            pltpu.VMEM((2, NKT, M, DH), BF16),
            pltpu.VMEM((NP, D, 2 * TN + PAD), BF16),
            pltpu.VMEM((NP, B, 2 * HG, SK, DH), BF16),
            pltpu.VMEM((NP, B, 2 * HG, SK, DH), BF16),
            pltpu.VMEM((NP, 2 * TN, D + PAD), BF16),
            pltpu.VMEM((NQS, HG, 4, DH // 2, RB), U32),
            pltpu.VMEM((NOS, HG, M, DH), BF16),
            pltpu.VMEM((NG0, M, TN), F32),
            pltpu.VMEM((M, D), F32),
            pltpu.VMEM((2, M, D), BF16),
            pltpu.SemaphoreType.DMA((NSEM,)),
        ],
        compiler_params=pltpu.CompilerParams(vmem_limit_bytes=100 * 1024 * 1024,
                                             disable_semaphore_checks=True),
    )(A_x.reshape(M, D), A_k_cache, A_v_cache, A_wq, A_wo,
      B_x.reshape(M, D), B_k_cache, B_v_cache, B_wq, B_wo)
    return out.reshape(B, SQ, 2 * D)
```

```python
import jax
import jax.numpy as jnp
from jax import lax
import jax.experimental.pallas as pl
import jax.experimental.pallas.tpu as pltpu

B, SQ, D = 16, 32, 1024
H, SK, DH = 32, 32, 128
M = B * SQ
HG = 4
TN = HG * DH
NP = 8
NPB = NP // 2
RB = 4 * SQ
NKT = D // DH
PAD = 128
SCALE = DH ** -0.5
F32 = jnp.float32
BF16 = jnp.bfloat16
U32 = jnp.uint32
P0 = 3

OQ = ((0, 256, 0, 512), (0, 256, 512, 512), (256, 256, 0, 512), (256, 256, 512, 512))
TAIL = (128, 64, 32, 32)
KPROG = ((1, 0, 0, 0, 0), (1, 1, 1, 0, 0), (2, 1, 1, 1, 1), (3, 3, 2, 2, 2), (5, 5, 4, 4, 4),
         (8, 8, 8, 8, 7), (8, 8, 8, 8, 8))
NG0 = len(KPROG[0])
NPH = len(KPROG)


def _chain(blocks, fills, prev):
    ops = []
    for b, f in zip(blocks, fills):
        ops += [("S", b, None) if prev is None else ("C", b, prev), f]
        prev = b
    return ops


def _q(g):
    return [("Q", g, h) for h in range(HG)]


def _o(g):
    return [("O", g, q) for q in OQ]


_BLK = [(g, c) for g in range(2) for c in range(4)]
FIRST_OPS = _chain(_BLK, _q(NG0) + _o(0), None)
AO_OPS = _chain(_BLK, _o(-1) + _o(0), (-1, 3))
PAIR_OPS = (_q(0) + _q(1)[:1]
            + [("C", (0, 0), (-1, 3)), _q(1)[1], _o(-1)[0], ("C", (0, 1), (0, 0)), _q(1)[2], _o(-1)[1],
               ("C", (0, 2), (0, 1)), _q(1)[3], _o(-1)[2]]
            + _chain(_BLK[3:], _o(-1)[3:] + _o(0), (0, 2)))
LAST_OPS = [("P", None, (-1, 3))] + _o(-1)

SEM_PAIR = NPH - 1
SEM_OUT = SEM_PAIR + NP + 1
NSEM = SEM_OUT + 1


def _out_pieces(q):
    r0, nr, c0, nc = q
    if q != OQ[-1]:
        return [q]
    last = c0 + nc - DH
    return ([(r0, nr, c, DH) for c in range(c0, last, DH)]
            + [(r0 + sum(TAIL[:i]), TAIL[i], last, DH) for i in range(len(TAIL))])


def _kernel(ax, ak, av, awq, awo, bx, bk, bv, bwq, bwo, out,
            x_buf, wq0_buf, wq_buf, k_buf, v_buf, wo_buf, qt_buf, o_buf, p_buf, qacc, acc, stage, sems):
    srcs = ((ax, ak, av, awq, awo), (bx, bk, bv, bwq, bwo))
    copy = pltpu.make_async_copy

    def cp(kind, sp, hf, n, p, sem):
        _, k, v, wq, wo = srcs[sp // NPB]
        lg = 2 * (sp % NPB) + hf
        if kind == "wq":
            return copy(wq.at[:, pl.ds(lg * TN, n * TN)], wq_buf.at[p, :, pl.ds(hf * TN, n * TN)], sem)
        if kind == "k":
            return copy(k.at[:, pl.ds(lg * HG, n * HG)], k_buf.at[p, :, pl.ds(hf * HG, n * HG)], sem)
        if kind == "v":
            return copy(v.at[:, pl.ds(lg * HG, n * HG)], v_buf.at[p, :, pl.ds(hf * HG, n * HG)], sem)
        return copy(wo.at[pl.ds(lg * TN, n * TN), :], wo_buf.at[p, pl.ds(hf * TN, n * TN), pl.ds(0, D)], sem)

    def cp_x(br, a, b, sem):
        ks = pl.ds(a * DH, (b - a) * DH)
        return copy(srcs[br][0].at[:, ks], x_buf.at[br, :, ks], sem)

    def kranges(i):
        return list(zip(KPROG[i - 1] if i else (0,) * NG0, KPROG[i]))

    def cp_chunk(i):
        kr = kranges(i)
        xa, xb = max(a for a, _ in kr), max(b for _, b in kr)
        cps = [cp_x(0, xa, xb, sems.at[i])] if xb > xa else []
        g = 0
        while g < NG0:
            n = 1
            while g + n < NG0 and kr[g + n] == kr[g]:
                n += 1
            a, b = kr[g]
            if b > a:
                ks, ns = pl.ds(a * DH, (b - a) * DH), pl.ds(g * TN, n * TN)
                cps.append(copy(awq.at[ks, ns], wq0_buf.at[ks, ns], sems.at[i]))
            g += n
        return cps

    def cp_pair(sp, p, with_wq):
        sem = sems.at[SEM_PAIR + p]
        return ([cp(kind, sp, 0, 2, p, sem) for kind in (("wq", "k", "v") if with_wq else ("k", "v"))]
                + [cp("wo", sp - 1, 1, 1, p - 1, sem), cp("wo", sp, 0, 1, p, sem)])

    def cp_xb():
        return cp_x(1, 0, NKT, sems.at[SEM_PAIR + NPB])

    def cp_out(br, r0, nr, c0, nc):
        rows = pl.ds(r0, nr)
        return copy(stage.at[br, rows, pl.ds(c0, nc)], out.at[rows, pl.ds(br * D + c0, nc)], sems.at[SEM_OUT])

    def wait_all(cps):
        for c in cps:
            c.wait()

    phase_cps = [cp_chunk(i) for i in range(NPH)]
    phase_cps[-1] += [cp(kind, sp, hf, n, sp, sems.at[SEM_PAIR]) for kind, sp, hf, n in
                      (("k", 0, 0, 2), ("wq", NG0 // 2, NG0 % 2, 1), ("v", 0, 0, 2), ("wo", 0, 0, 1))]
    last_cps = [cp("wo", NP - 1, 1, 1, NP - 1, sems.at[SEM_PAIR + NP])]
    for cps in (phase_cps + [([cp_xb()] if p == NPB else []) + cp_pair(p, p, p >= P0) for p in range(1, NP)]
                + [last_cps]):
        for c in cps:
            c.start()

    lane = lax.broadcasted_iota(jnp.int32, (SK, 128), 1) // SK
    lane2 = lax.broadcasted_iota(jnp.int32, (SK // 2, 128), 1) // SK
    zero2 = jnp.zeros((SK // 2, 128), U32)
    packed = lambda a: pltpu.bitcast(a, U32)
    unpacked = lambda a: pltpu.bitcast(a, BF16)
    keep = lambda j, a: jnp.where(lane2 != j, zero2, a)
    drop = lambda j, a: jnp.where(lane2 == j, zero2, a)
    sel = lambda j, a, b: jnp.where(lane2 == j, a, b)

    def store_q(slot, h, q):
        for c in range(4):
            qt_buf[slot, h, c] = packed(q[c * RB:(c + 1) * RB].T.astype(BF16))

    def softmax_t(ss):
        pts = []
        for s in ss:
            mx = jnp.max(s, axis=0, keepdims=True)
            e = jnp.exp((s - mx) * SCALE)
            l = jnp.sum(e, axis=0, keepdims=True)
            pts.append(e * (1.0 / l))
        return packed(jnp.concatenate(pts, axis=0).T.astype(BF16))

    def dot(a, rows):
        return jnp.dot(unpacked(a), unpacked(jnp.concatenate(rows, axis=0)), preferred_element_type=F32)

    def run(ops, p, br, qslot, first, emit, pr):
        pair_of = lambda g: p + g // 2 if g // 2 else p
        for op, a, b in ops:
            if op == "Q":
                g, h = a, b
                q = jnp.dot(x_buf[br, :, pl.ds(0, D)], wq_buf[pair_of(g), :, pl.ds((g % 2) * TN + h * DH, DH)],
                            preferred_element_type=F32)
                store_q(qslot(g), h, q)
                continue
            if op == "O":
                g, (r0, nr, c0, nc) = a, b
                rows, cols = pl.ds(r0, nr), pl.ds(c0, nc)
                o = jnp.concatenate([o_buf[g % 2, h, rows, :] for h in range(HG)], axis=1)
                r = jnp.dot(o, wo_buf[pair_of(g), pl.ds((g % 2) * TN, TN), cols], preferred_element_type=F32)
                if g != 0 or first is False:
                    r = acc[rows, cols] + r
                elif first is not True:
                    r = jnp.where(first, 0.0, acc[rows, cols]) + r
                acc[rows, cols] = r
                if g < 0 and emit is not None:
                    emit(b, r)
                continue
            if a is not None:
                gs, cs = a
                kk = lambda i, j: packed(k_buf[pair_of(gs), cs * 4 + j, (gs % 2) * HG + i])
                qt = lambda i, r: qt_buf[qslot(gs), i, cs, pl.ds(r * (SK // 2), SK // 2), :]
            if b is not None:
                gp, cv = b
                vv = lambda i, r: packed(v_buf[pair_of(gp), cv * 4 + i, (gp % 2) * HG + r])
                pc = [pr[i * (SQ // 2):(i + 1) * (SQ // 2)] for i in range(4)]

                def put_o(i, j, o):
                    o_buf[gp % 2, j, pl.ds(cv * RB + i * SQ, SQ), :] = o.astype(BF16)
            if op == "S":
                ss = []
                for i in range(4):
                    st = dot(jnp.concatenate([kk(i, j) for j in range(4)], axis=0), [qt(i, r) for r in range(4)])
                    ss.append(jnp.where(lane == 0, st[0:32], jnp.where(
                        lane == 1, st[32:64], jnp.where(lane == 2, st[64:96], st[96:128]))))
                pr = softmax_t(ss)
            elif op == "P":
                for i in range(4):
                    o = dot(jnp.concatenate([keep(j, pc[i]) for j in range(4)], axis=0),
                            [vv(i, r) for r in range(4)])
                    for j in range(4):
                        put_o(i, j, o[j * SQ:(j + 1) * SQ])
            else:
                ss = [dot(sel(0, kk(i, 0), sel(1, kk(i, 1), sel(2, kk(i, 2), kk(i, 3)))),
                          [keep(r, qt(i, r)) for r in range(4)]) for i in range(4)]
                od = [dot(pc[i], [keep(r, vv(i, r)) for r in range(4)]) for i in range(4)]
                for j in range(4):
                    for i in range(4):
                        t = dot(sel(j, pc[i], kk(i, j)),
                                [drop(j, vv(i, r)) if r == j else keep(j, qt(i, r)) for r in range(4)])
                        put_o(i, j, jnp.where(lane == j, od[i], t))
                        ss[i] = jnp.where(lane == j, ss[i] + t, ss[i])
                pr = softmax_t(ss)
        return pr

    for ph in range(NPH):
        wait_all(phase_cps[ph])
        for g, (a, b) in enumerate(kranges(ph)):
            if b == a:
                continue
            ks = pl.ds(a * DH, (b - a) * DH)
            r = jnp.dot(x_buf[0, :, ks], wq0_buf[ks, pl.ds(g * TN, TN)], preferred_element_type=F32)
            if a > 0:
                r = r + qacc[g]
            if b < NKT:
                qacc[g] = r
            else:
                for h in range(HG):
                    store_q(g, h, r[:, h * DH:(h + 1) * DH])
    p_buf[...] = run(FIRST_OPS, 0, 0, lambda g: g, True, None, None)

    def ao_step(p, carry):
        wait_all(cp_pair(1, p, False))
        p_buf[...] = run(AO_OPS, p, 0, lambda g: 2 * p + g, False, None, p_buf[...])
        return carry

    lax.fori_loop(1, P0, ao_step, 0)

    def pair_step(p, carry):
        @pl.when(p == NPB)
        def _():
            cp_xb().wait()

        wait_all(cp_pair(1, p, True))

        @pl.when(p == NPB + 1)
        def _():
            cp_out(0, 0, M, 0, D).start()

        def emit(q, r):
            stage[lax.shift_right_logical(p - 1, 2), pl.ds(q[0], q[1]), pl.ds(q[2], q[3])] = r.astype(BF16)

        p_buf[...] = run(PAIR_OPS, p, lax.shift_right_logical(p, 2), lambda g: g, p == NPB, emit, p_buf[...])
        return carry

    lax.fori_loop(P0, NP, pair_step, 0)

    def emit_last(q, r):
        for r0, nr, c0, nc in _out_pieces(q):
            stage[1, pl.ds(r0, nr), pl.ds(c0, nc)] = (
                r[r0 - q[0]:r0 - q[0] + nr, c0 - q[2]:c0 - q[2] + nc].astype(BF16))
            cp_out(1, r0, nr, c0, nc).start()

    wait_all(last_cps)
    run(LAST_OPS, NP, 1, None, False, emit_last, p_buf[...])
    cp_out(0, 0, M, 0, D).wait()
    for q in OQ:
        for piece in _out_pieces(q):
            cp_out(1, *piece).wait()


@jax.jit
def pallas_concat_heads__mha_block_cached__mha_block_cached__near_ridge_kernel(
    A_x: jax.Array,
    A_k_cache: jax.Array,
    A_v_cache: jax.Array,
    A_wq: jax.Array,
    A_wo: jax.Array,
    B_x: jax.Array,
    B_k_cache: jax.Array,
    B_v_cache: jax.Array,
    B_wq: jax.Array,
    B_wo: jax.Array,
):
    any_spec = pl.BlockSpec(memory_space=pl.ANY)
    out = pl.pallas_call(
        _kernel,
        out_shape=jax.ShapeDtypeStruct((M, 2 * D), BF16),
        in_specs=[any_spec] * 10,
        out_specs=any_spec,
        scratch_shapes=[
            pltpu.VMEM((2, M, D + PAD), BF16),
            pltpu.VMEM((D, NG0 * TN + PAD), BF16),
            pltpu.VMEM((NP, D, 2 * TN + PAD), BF16),
            pltpu.VMEM((NP, B, 2 * HG, SK, DH), BF16),
            pltpu.VMEM((NP, B, 2 * HG, SK, DH), BF16),
            pltpu.VMEM((NP, 2 * TN, D + PAD), BF16),
            pltpu.VMEM((2 * P0, HG, 4, DH // 2, RB), U32),
            pltpu.VMEM((2, HG, M, DH), BF16),
            pltpu.VMEM((RB // 2, 128), U32),
            pltpu.VMEM((NG0, M, TN), F32),
            pltpu.VMEM((M, D), F32),
            pltpu.VMEM((2, M, D), BF16),
            pltpu.SemaphoreType.DMA((NSEM,)),
        ],
        compiler_params=pltpu.CompilerParams(vmem_limit_bytes=100 * 1024 * 1024,
                                             disable_semaphore_checks=True),
    )(A_x.reshape(M, D), A_k_cache, A_v_cache, A_wq, A_wo,
      B_x.reshape(M, D), B_k_cache, B_v_cache, B_wq, B_wo)
    return out.reshape(B, SQ, 2 * D)
```
